```python
import os as _os
_os.environ.setdefault("JAX_PLATFORMS", "cpu")
import jax
import jax.numpy as jnp

def _softmax(x, axis=-1):
    return jax.nn.softmax(x, axis=axis)
def _gelu(x):
    return jax.nn.gelu(x, approximate=True)
def _silu(x):
    return jax.nn.silu(x)
def _sigmoid(x):
    return jax.nn.sigmoid(x)
def _layernorm(x, axis=-1, eps=1e-5):
    m = jnp.mean(x, axis=axis, keepdims=True)
    v = jnp.var(x, axis=axis, keepdims=True)
    return (x - m) / jnp.sqrt(v + eps)
def _scatter_add(tgt, idx, src, axis=0):
    return tgt.at[idx].add(src)
def _segment_sum(src, seg, n):
    return jax.ops.segment_sum(src, seg, n)
class _Rng:
    def __init__(self, key):
        self._k = key
    def _next(self):
        self._k, sub = jax.random.split(self._k)
        return sub
    def normal(self, shape):
        return jax.random.normal(self._next(), shape, dtype=jnp.bfloat16)
    def randint(self, lo, hi, shape):
        return jax.random.randint(self._next(), shape, lo, hi, dtype=jnp.int32)
    def uniform(self, shape, lo=0.0, hi=1.0):
        return jax.random.uniform(self._next(), shape, jnp.bfloat16, lo, hi)
    def permutation(self, n):
        return jax.random.permutation(self._next(), n)


kernel_name = 'recurrent_scan__ssm_conv_s4__mixer_s_mlp__prompt'

def setup_inputs():
    _rng = _Rng(jax.random.key(int.from_bytes(__import__("os").urandom(4), "little")))
    _w = (lambda a: (lambda t: t.astype(jnp.bfloat16) if jnp.issubdtype(t.dtype, jnp.floating) else t)(jnp.asarray(a)))
    def _A_setup():
        B, L, D, N = 1, 2048, 512, 128
        A_re = -jnp.exp((lambda *s: _rng.normal(s) * 0.1)(D, N))
        A_im = jnp.pi * (lambda *s: _rng.normal(s) * 0.1)(D, N)
        B_re = (lambda *s: _rng.normal(s) * 0.1)(D, N)
        B_im = (lambda *s: _rng.normal(s) * 0.1)(D, N)
        C_re = (lambda *s: _rng.normal(s) * 0.1)(D, N)
        C_im = (lambda *s: _rng.normal(s) * 0.1)(D, N)
        log_dt = (lambda *s: _rng.normal(s) * 0.1)(D) * 0.5 - 4.0
        Dskip = (lambda *s: _rng.normal(s) * 0.05)(D)
        return {
            "u": _w((lambda *s: _rng.normal(s) * 0.05)(B, L, D)),
            "A_re": _w(A_re),
            "A_im": _w(A_im),
            "B_re": _w(B_re),
            "B_im": _w(B_im),
            "C_re": _w(C_re),
            "C_im": _w(C_im),
            "log_dt": _w(log_dt),
            "Dskip": _w(Dskip),
        }
    _A_in = _A_setup()

    def _B_setup():
        B, S, D, F = 1, 2048, 512, 1376
        return {
            "x":  _w((lambda *s: _rng.normal(s) * 0.05)(B, S, D)),
            "w1": _w((lambda *s: _rng.normal(s) * 0.8)(D, D) * (D ** -0.5)),
            "w2": _w((lambda *s: _rng.normal(s) * 0.8)(D, D) * (D ** -0.5)),
            "w3": _w((lambda *s: _rng.normal(s) * 0.8)(D, F) * (D ** -0.5)),
            "w4": _w((lambda *s: _rng.normal(s) * 0.8)(F, D) * (F ** -0.5)),
        }
    _B_in = _B_setup()

    return {
        "A_u": _A_in["u"],
        "A_A_re": _A_in["A_re"],
        "A_A_im": _A_in["A_im"],
        "A_B_re": _A_in["B_re"],
        "A_B_im": _A_in["B_im"],
        "A_C_re": _A_in["C_re"],
        "A_C_im": _A_in["C_im"],
        "A_log_dt": _A_in["log_dt"],
        "A_Dskip": _A_in["Dskip"],
        "B_x": _B_in["x"],
        "B_w1": _B_in["w1"],
        "B_w2": _B_in["w2"],
        "B_w3": _B_in["w3"],
        "B_w4": _B_in["w4"],
    }

def reference(A_u, A_A_re, A_A_im, A_B_re, A_B_im, A_C_re, A_C_im, A_log_dt, A_Dskip, B_x, B_w1, B_w2, B_w3, B_w4):
    def _A_ref(u, A_re, A_im, B_re, B_im, C_re, C_im, log_dt, Dskip):
        Bsz, L, D = u.shape
        dt = jnp.exp(log_dt)[:, None]
        A = A_re + 1j * A_im
        Bc = B_re + 1j * B_im
        Cc = C_re + 1j * C_im
        logdA = dt * A
        dB = dt * Bc
        l = (lambda x, dt: x.astype(dt))(jnp.arange(L), A_re.dtype)
        P = jnp.exp(logdA[:, :, None] * l[None, None, :])
        K = jnp.einsum("dn,dnl,dn->dl", Cc, P, dB).real
        L2 = 2 * L
        Kp = jnp.pad(K, ((0, 0), (0, L)))
        up = (lambda x, *d: x.transpose(*d))(u, 0, 2, 1)
        up = jnp.pad(up, ((0, 0), (0, 0), (0, L)))
        Kf = (lambda x, axes=(-2,-1): jnp.fft.rfft2(x.astype(jnp.float32), axes=axes))(Kp[:, None, :], axes=(-2, -1))
        Uf = (lambda x, axes=(-2,-1): jnp.fft.rfft2(x.astype(jnp.float32), axes=axes))(up[:, :, None, :], axes=(-2, -1))
        Yf = Uf * Kf[None, :, :, :]
        y = (lambda x, s, axes=(-2,-1): jnp.fft.irfft2(x, s=s, axes=axes).astype(jnp.bfloat16))(Yf, (1, L2), axes=(-2, -1))[:, :, 0, :L]
        y = (lambda x, *d: x.transpose(*d))(y, 0, 2, 1) + u * Dskip[None, None, :]
        return y

    def _B_ref(x, w1, w2, w3, w4):
        B, S, D = x.shape
        h = _gelu(_layernorm(x, axis=-1) @ w1)
        c = D // 4
        g0 = jnp.pad(h[:, :, 0*c:1*c], ((0, 0), (1, 0), (0, 0)))[:, :S, :]
        g1 = jnp.pad(h[:, :, 1*c:2*c], ((0, 0), (0, 1), (0, 0)))[:, 1:, :]
        g2 = jnp.pad(h[:, :, 2*c:3*c], ((0, 0), (2, 0), (0, 0)))[:, :S, :]
        g3 = jnp.pad(h[:, :, 3*c:   ], ((0, 0), (0, 2), (0, 0)))[:, 2:, :]
        hs = jnp.concatenate([g0, g1, g2, g3], axis=-1) @ w2
        x1 = x + hs
        h2 = _gelu(_layernorm(x1, axis=-1) @ w3) @ w4
        return x1 + h2

    x = A_u
    xn = _layernorm(x, axis=-1)
    s = _A_ref(xn, A_A_re, A_A_im, A_B_re, A_B_im, A_C_re, A_C_im, A_log_dt, A_Dskip)
    g = _silu(_B_ref(xn, B_w1, B_w2, B_w3, B_w4))
    return x + s * g
```

```python
import functools
import jax
import jax.numpy as jnp
from jax import lax
import jax.experimental.pallas as pl
import jax.experimental.pallas.tpu as pltpu

L, D, N, F = 2048, 512, 128, 1376
T = 64
C = L // T
P = D // 2
SR = C + 1
BR = 9
F32, BF16 = jnp.float32, jnp.bfloat16


def _ln(x):
    m = jnp.mean(x, axis=-1, keepdims=True)
    xc = x - m
    v = jnp.mean(xc * xc, axis=-1, keepdims=True)
    return xc * lax.rsqrt(v + 1e-5)


def _gelu(x):
    c = 0.7978845608028654
    return 0.5 * x * (1.0 + jnp.tanh(x * (c + (c * 0.044715) * (x * x))))


def _cmul(ar, ai, br, bi):
    return ar * br - ai * bi, ar * bi + ai * br


def _mm(a, b):
    return jnp.dot(a, b, preferred_element_type=F32)


def _col(row_ref):
    r = row_ref[...].astype(F32).reshape(1, D)
    return jnp.broadcast_to(r, (128, D)).T


def kernel(x_ref, are_ref, aim_ref, bre_ref, bim_ref, cre_ref, cim_ref, ldt_ref, dsk_ref,
           w1_ref, w2_ref, w3_ref, w4_ref, o_ref,
           xn_s, a1_s, up_s, base_s, q_s, zr_s, zi_s, sr_s, si_s, y_s, h0_s, h1_s, h2_s, h3_s, dk_s, g_s, a2_s, w1_s, w2_s, w3_s, *ss):
    i32 = lambda v: pltpu.bitcast(v, jnp.int32)
    b16 = lambda v: pltpu.bitcast(v, BF16)
    NG = 16
    def sref(k, d): return ss[k * (D // NG) + d // NG]
    w1_s[...] = i32(w1_ref[...])
    w2_s[...] = i32(w2_ref[...])
    w3_s[0:F // 2, :] = i32(w3_ref[...])
    half = lambda i, n: pl.ds(i * n // 2 if isinstance(i, int) else pl.multiple_of(i * (n // 2), n // 2), n // 2)
    dt = jnp.exp(_col(ldt_ref))
    a = dt * are_ref[...].astype(F32)
    b = dt * aim_ref[...].astype(F32)
    e = jnp.exp(a)
    zr, zi = e * jnp.cos(b), e * jnp.sin(b)
    wr, wi = _cmul(cre_ref[...].astype(F32), cim_ref[...].astype(F32),
                   dt * bre_ref[...].astype(F32), dt * bim_ref[...].astype(F32))
    dk_s[...] = jnp.sum(wr.T, axis=0, keepdims=True) + dsk_ref[...].astype(F32).reshape(1, D)
    xr, xi = _cmul(wr, wi, zr, zi)
    m = jnp.maximum(jnp.abs(xr), jnp.abs(xi))
    ms = jnp.where(m > 0, m, 1.0)
    ur, ui = xr / ms, xi / ms
    t = jnp.sqrt(0.5 * (jnp.sqrt(ur * ur + ui * ui) + jnp.abs(ur)))
    o = ui / jnp.where(t > 0, 2.0 * t, 1.0)
    sm = jnp.sqrt(ms)
    vr = sm * jnp.where(ur >= 0, t, jnp.abs(o))
    vi = sm * jnp.where(ur >= 0, o, jnp.where(ui >= 0, t, -t))
    for d in range(0, D, NG):
        sref(0, d)[pl.ds(0, NG, stride=SR), :] = vr[d:d + NG]
        sref(1, d)[pl.ds(0, NG, stride=SR), :] = -vi[d:d + NG]
    z2 = _cmul(zr, zi, zr, zi)
    z4 = _cmul(*z2, *z2)
    z8 = _cmul(*z4, *z4)
    z16 = _cmul(*z8, *z8)
    z32 = _cmul(*z16, *z16)
    z64 = _cmul(*z32, *z32)
    rows = [(vr, vi)]
    rows.append(_cmul(vr, vi, zr, zi))
    rows += [_cmul(*r, *z2) for r in rows]
    rows += [_cmul(*r, *z4) for r in rows]
    for s, (r, i) in enumerate(rows):
        base_s[0, pl.ds(s, D, stride=BR), :] = r
        base_s[1, pl.ds(s, D, stride=BR), :] = i
    for k, (r, i) in enumerate((z8, z16, z32, z64)):
        q_s[2 * k] = r
        q_s[2 * k + 1] = i

    for hb in (h0_s, h1_s, h2_s, h3_s):
        hb[0:8, :] = jnp.zeros((8, 128), F32)
        hb[L + 8:L + 16, :] = jnp.zeros((8, 128), F32)


    RB = 256
    NC = RB // T
    GP = 32
    hbs = (h0_s, h1_s, h2_s, h3_s)

    def rows(i, n):
        return pl.ds(i * n if isinstance(i, int) else pl.multiple_of(i * n, n), n)

    def pre(c):
        xn = _ln(x_ref[rows(c, T), :].astype(F32))
        xn_s[rows(c, T), :] = xn
        a1_s[half(c, T), :] = i32(_ln(xn).astype(BF16))
        for pb in range(2):
            tile = jnp.concatenate([xn[:, pb * 128:(pb + 1) * 128],
                                    xn[:, P + pb * 128:P + (pb + 1) * 128]], axis=0)
            up_s[pl.ds(pb * 128 * SR + c, 128, stride=SR), :] = tile.T

    def mix1(i, side):
        for g, hb in enumerate(hbs):
            h = _gelu(_mm(b16(a1_s[half(i, RB), :]), b16(w1_s[:, g * 128:(g + 1) * 128])))
            hb[pl.ds(i * RB + 8, RB), :] = h
            side(g, 4)

    lane = lax.broadcasted_iota(jnp.int32, (C, 128), 1)
    lo = lane < T
    rev = jnp.where(lo, T - 1 - lane, 3 * T - 1 - lane)

    def table(d):
        br, bi = base_s[0, pl.ds(d * BR, 8), :], base_s[1, pl.ds(d * BR, 8), :]
        bq = lambda k: (q_s[2 * k, pl.ds(d, 8, stride=0), :], q_s[2 * k + 1, pl.ds(d, 8, stride=0), :])
        cur = (br, bi), _cmul(br, bi, *bq(0))
        q = bq(1)
        rs, ms_ = [], []
        for k in range(4):
            rs.append(jnp.concatenate([cur[0][0], cur[1][0]], axis=0).astype(BF16))
            ms_.append(jnp.concatenate([cur[0][1], cur[1][1]], axis=0).astype(BF16))
            if k < 3:
                cur = _cmul(*cur[0], *q), _cmul(*cur[1], *q)
        return jnp.concatenate(rs, axis=0), jnp.concatenate(ms_, axis=0)

    def ssm_in(p):
        ar, ai = table(p)
        br, bi = table(p + P)
        tr = jnp.concatenate([ar, br], axis=0)
        ti = jnp.concatenate([ai, bi], axis=0)
        zr_s[p] = i32(tr)
        zi_s[p] = i32(ti)
        u = jnp.take_along_axis(up_s[pl.ds(p * SR, C), :], rev, axis=1)
        lhs = jnp.concatenate([jnp.where(lo, u, 0.0), jnp.where(lo, 0.0, u)], axis=0).astype(BF16)
        for ref, tab in ((0, tr), (1, ti)):
            s = _mm(lhs, tab)
            sref(ref, p)[pl.ds(p % NG * SR + 1, C), :] = s[:C]
            sref(ref, p + P)[pl.ds(p % NG * SR + 1, C), :] = s[C:]

    def scan(d0):
        G = 8
        qr, qi = q_s[6, pl.ds(d0, G), :], q_s[7, pl.ds(d0, G), :]
        at = lambda c: pl.ds(d0 % NG * SR + c, G, stride=SR)
        sr_s, si_s = sref(0, d0), sref(1, d0)
        hr, hn = sr_s[at(1), :], -si_s[at(1), :]
        si_s[at(1), :] = hn
        for c in range(2, C):
            hr, hn = (qr * hr + qi * hn + sr_s[at(c), :], qr * hn - qi * hr - si_s[at(c), :])
            sr_s[at(c), :] = hr
            si_s[at(c), :] = hn

    lo8 = lax.broadcasted_iota(jnp.int32, (1, 128), 1) < T
    row8 = lax.broadcasted_iota(jnp.int32, (8, 128), 0)
    laneT = lax.broadcasted_iota(jnp.int32, (T, 128), 1)

    def ssm_out(p):
        def h(ref):
            return jnp.concatenate([sref(ref, d)[pl.ds(d % NG * SR, C), :] for d in (p, p + P)], axis=0).astype(BF16)
        lhs = jnp.concatenate([h(0), h(1)], axis=1)
        tab = jnp.concatenate([b16(zr_s[p]), b16(zi_s[p])], axis=1)
        r = lax.dot_general(lhs, tab, (((1,), (1,)), ((), ())), preferred_element_type=F32)
        y = jnp.where(lo, r[:C], r[C:])
        y = jnp.concatenate([jnp.where(row8 > 0, y[:8], 0.0), y[8:]], axis=0)
        k0 = jnp.broadcast_to(jnp.where(lo8, r[0:1], 0.0), (T, 128))
        k1 = jnp.broadcast_to(jnp.where(lo8, 0.0, r[C:C + 1]), (T, 128))
        t0 = jnp.where(laneT < T, pltpu.roll(k0, 1, 1, stride=1, stride_axis=0), 0.0)
        t1 = jnp.where(laneT < T, 0.0, pltpu.roll(k1, 1, 1, stride=1, stride_axis=0))
        toe = jnp.concatenate([t0, t1], axis=0).astype(BF16)
        y_s[pl.ds(p * SR, C), :] = y + _mm(up_s[pl.ds(p * SR, C), :].astype(BF16), toe)

    def ssm_side(gi, gs, go):
        work = []
        for u in range(GP):
            if gi is not None:
                work.append(functools.partial(ssm_in, gi * GP + u))
            if go is not None:
                work.append(functools.partial(ssm_out, go * GP + u))
            if gs is not None and u % 16 == 0:
                work.append(functools.partial(scan, pl.multiple_of(gs * GP + (u // 16) * P, GP)))

        def side(k, n):
            for f in work[k * len(work) // n:(k + 1) * len(work) // n]:
                f()
        return side

    FC = [(f, min(f + 128, F)) for f in range(0, F, 128)]

    def loop(n, body):
        for i in range(n):
            body(i)

    def mm2q(i, k):
        r0 = i * RB
        hs = jnp.concatenate([h0_s[pl.ds(r0 + 7, RB), :], h1_s[pl.ds(r0 + 9, RB), :],
                              h2_s[pl.ds(r0 + 6, RB), :], h3_s[pl.ds(r0 + 10, RB), :]], axis=1).astype(BF16)
        cs = slice(k * 128, (k + 1) * 128)
        g_s[rows(i, RB), cs] = xn_s[rows(i, RB), cs] + _mm(hs, b16(w2_s[:, cs]))

    def ln2(i):
        a2_s[half(i, RB), :] = i32(_ln(g_s[rows(i, RB), :]).astype(BF16))

    def mlp(i, side):
        n = len(FC)
        d3 = lambda k: lax.dot_general(b16(a2_s[half(i, RB), :]), b16(w3_s[FC[k][0] // 2:FC[k][1] // 2, :]),
                                       (((1,), (1,)), ((), ())), preferred_element_type=F32)
        t = d3(0)
        for k, (f0, f1) in enumerate(FC):
            tn = d3(k + 1) if k + 1 < n else None
            side(k, n)
            g = g_s[rows(i, RB), :] + _mm(_gelu(t).astype(BF16), w4_ref[f0:f1, :])
            if tn is None:
                g = g * jax.nn.sigmoid(g)
            g_s[rows(i, RB), :] = g
            t = tn

    for c in range(NC):
        pre(c)
    with jax.named_scope('s_mix'):
      loop(7, lambda i: mix1(i, lambda k, n: pre((i + 1) * NC + k)))
      mix1(7, lambda k, n: ssm_in(k))
    with jax.named_scope('s_2'):
      for i in range(8):
        for k in range(4):
            mm2q(i, k)
            ln2(i - 1) if (k == 0 and i) else None
            ssm_in(4 + i * 4 + k)
      ln2(7)
    def plan():
        w = {j: [] for j in range(8)}
        ins = list(range(36, P))
        state = dict(i=36, s=0, o=0)
        total = 8 * len(FC)
        sched = []
        for step in range(total):
            items = []
            for _ in range(3 if step < total - 8 else 4):
                if state['i'] < P:
                    items.append(functools.partial(ssm_in, state['i'])); state['i'] += 1
            if state['s'] + 24 <= state['i'] or (state['i'] == P and state['s'] < P and step >= 75):
                s0 = state['s']; state['s'] += 8
                items.append(functools.partial(scan, s0)); items.append(functools.partial(scan, s0 + P))
            for _ in range(3 if state['i'] < P else 5):
                if state['o'] + 24 < state['s'] or (state['s'] == P and state['o'] < P):
                    items.append(functools.partial(ssm_out, state['o'])); state['o'] += 1
            sched.append(items)
        assert state['o'] == P, state
        return sched
    sched = plan()
    with jax.named_scope('s_mlp'):
      for j in range(8):
        mlp(j, lambda k, n: [f() for f in sched[j * n + k]])

    def post(c):
        for pb in range(2):
            tt = y_s[pl.ds(pb * 128 * SR + c, 128, stride=SR), :].T
            for e in range(2):
                cs = slice(e * P + pb * 128, e * P + (pb + 1) * 128)
                s = tt[e * T:(e + 1) * T] + xn_s[rows(c, T), cs] * dk_s[:, cs]
                o_ref[rows(c, T), cs] = (x_ref[rows(c, T), cs].astype(F32) + s * g_s[rows(c, T), cs]).astype(BF16)
    with jax.named_scope('s_post'):
      (lambda n, b: lax.fori_loop(0, n, lambda i, c: (b(i), c)[1], 0))(C // 4, lambda i: [post(4 * i + k) for k in range(4)])


@jax.jit
def pallas_recurrent_scan__ssm_conv_s4__mixer_s_mlp__prompt_kernel(A_u, A_A_re, A_A_im, A_B_re, A_B_im, A_C_re, A_C_im, A_log_dt, A_Dskip, B_x, B_w1, B_w2, B_w3, B_w4):
    del B_x
    V = pltpu.VMEM
    out = pl.pallas_call(
        kernel,
        out_shape=jax.ShapeDtypeStruct((L, D), BF16),
        scratch_shapes=[
            V((L, D), F32), V((L // 2, D), jnp.int32), V((P * SR, 128), F32),
            V((2, D * BR, 128), F32), V((8, D, 128), F32),
            V((P, 64, 128), jnp.int32), V((P, 64, 128), jnp.int32),
            V((8, 128), F32), V((8, 128), F32), V((P * SR, 128), F32),
            V((L + 16, 128), F32), V((L + 16, 128), F32), V((L + 16, 128), F32), V((L + 16, 128), F32),
            V((1, D), F32), V((L, D), F32), V((L // 2, D), jnp.int32), V((256, D), jnp.int32), V((256, D), jnp.int32), V((F // 2, D), jnp.int32), *[V((16 * SR, 128), F32)] * 64,
        ],
        compiler_params=pltpu.CompilerParams(flags={'XLA_TPU_FORCE_LP_LLO_SCHEDULER':True}, vmem_limit_bytes=110 * 2**20),
        name="ssm_mixer",
    )(A_u.reshape(L, D), A_A_re, A_A_im, A_B_re, A_B_im, A_C_re, A_C_im, A_log_dt, A_Dskip,
      B_w1, B_w2, B_w3.T, B_w4)
    return out.reshape(1, L, D)
```
